```python
import jax
import jax.numpy as jnp

def _softmax(x, axis=-1):
    return jax.nn.softmax(x, axis=axis)
def _gelu(x):
    return jax.nn.gelu(x, approximate=True)
def _silu(x):
    return jax.nn.silu(x)
def _sigmoid(x):
    return jax.nn.sigmoid(x)
def _layernorm(x, axis=-1, eps=1e-5):
    m = jnp.mean(x, axis=axis, keepdims=True)
    v = jnp.var(x, axis=axis, keepdims=True)
    return (x - m) / jnp.sqrt(v + eps)
def _scatter_add(tgt, idx, src, axis=0):
    return tgt.at[idx].add(src)
def _segment_sum(src, seg, n):
    return jax.ops.segment_sum(src, seg, n)
class _Rng:
    def __init__(self, key):
        self._k = key
    def _next(self):
        self._k, sub = jax.random.split(self._k)
        return sub
    def normal(self, shape):
        return jax.random.normal(self._next(), shape, dtype=jnp.bfloat16)
    def randint(self, lo, hi, shape):
        return jax.random.randint(self._next(), shape, lo, hi, dtype=jnp.int32)
    def uniform(self, shape, lo=0.0, hi=1.0):
        return jax.random.uniform(self._next(), shape, jnp.bfloat16, lo, hi)
    def permutation(self, n):
        return jax.random.permutation(self._next(), n)


kernel_name = 'standalone__gqa_block_cached__near_ridge'

def setup_inputs():
    _rng = _Rng(jax.random.key(int.from_bytes(__import__("os").urandom(4), "little")))
    _w = (lambda a: (lambda t: t.astype(jnp.bfloat16) if jnp.issubdtype(t.dtype, jnp.floating) else t)(jnp.asarray(a)))
    B, Sq, D = 16, 240, 640
    Hq, Hkv, Sk, Dh = 32, 32, 1024, 128
    assert Hq % Hkv == 0, (Hq, Hkv)
    return {
        "x": _w((lambda *s: _rng.normal(s) * 0.05)(B, Sq, D)),
        "k_cache": _w((lambda *s: _rng.normal(s) * 0.05)(B, Hkv, Sk, Dh)),
        "v_cache": _w((lambda *s: _rng.normal(s) * 0.05)(B, Hkv, Sk, Dh)),
        "wq": _w((lambda *s: _rng.normal(s) * 0.05)(D, Hq * Dh) * (D ** -0.5)),
        "wo": _w((lambda *s: _rng.normal(s) * 0.05)(Hq * Dh, D) * ((Hq * Dh) ** -0.5)),
    }

def reference(x, k_cache, v_cache, wq, wo):
    B, Sq, D = x.shape
    Hq, Dh = 32, 128
    Hkv = k_cache.shape[1]
    rep = Hq // Hkv
    q = (lambda x, *d: x.transpose(*d))((x @ wq).reshape(B, Sq, Hq, Dh), 0, 2, 1, 3)
    k = jnp.repeat(k_cache, rep, axis=1)
    v = jnp.repeat(v_cache, rep, axis=1)
    scores = jnp.einsum("bhqd,bhkd->bhqk", q, k) * (Dh ** -0.5)
    p = _softmax(scores, axis=-1)
    o = jnp.einsum("bhqk,bhkd->bhqd", p, v)
    return (lambda x, *d: x.transpose(*d))(o, 0, 2, 1, 3).reshape(B, Sq, Hq * Dh) @ wo
```

```python
import functools
import math

import jax
import jax.numpy as jnp
from jax import lax
import jax.experimental.pallas as pl
import jax.experimental.pallas.tpu as pltpu

DH = 128
HG = 4
W = HG * DH
NSLOT = 8
NH = 16
U = NH // HG
WARM_B = 2
LEAD_AT = (3, 7, 10, 13)

WARM_ORDER = "Q0 Q1 P0 Q2 P1 Q3 P2 P3 N0 C0".split()


def _main_order():
    toks = ["Q0"]
    for h in range(NH - 2):
        toks.append(f"Q{h + 1}")
        if (h + 2) % HG == 0:
            toks.append(f"A{(h + 2) // HG}")
        if h >= 2:
            toks.append(f"c{h - 2}")
            if (h - 2) % HG == HG - 1:
                toks.append(f"d{(h - 2) // HG}")
        toks.append(f"P{h}")
    n = NH
    return toks + [f"Q{n - 1}", f"c{n - 4}", f"P{n - 2}", f"c{n - 3}", f"P{n - 1}",
                   "N0", f"c{n - 2}", f"c{n - 1}!", f"d{U - 1}"]


def _kernel(x_hbm, k_hbm, v_hbm, wq_hbm, wo_hbm, o_hbm,
            xbuf, wqbuf, wobuf, kvbuf, qs, acc, outbuf,
            xsem, wqsem, wosem, kvsem, osem):
    B, Sq, D = x_hbm.shape
    G = k_hbm.shape[1] // HG
    NC = B * G
    J = WARM_B * G
    scale = (DH ** -0.5) * math.log2(math.e)

    def where_is(n):
        n = jnp.asarray(n, jnp.uint32)
        warm = n < J
        b = jnp.where(warm, n % WARM_B, n // G)
        g = jnp.where(warm, n // WARM_B, n % G)
        return b.astype(jnp.int32), g.astype(jnp.int32)

    def slot(n):
        return (jnp.asarray(n, jnp.uint32) % NSLOT).astype(jnp.int32)

    def x_cp(b):
        return pltpu.make_async_copy(x_hbm.at[b], xbuf.at[b], xsem.at[b % 2])

    def wq_cp(g):
        return pltpu.make_async_copy(
            wq_hbm.at[:, pl.ds(pl.multiple_of(g * W, W), W)], wqbuf.at[g], wqsem.at[g])

    def wo_cp(g):
        return pltpu.make_async_copy(
            wo_hbm.at[pl.ds(pl.multiple_of(g * W, W), W), :], wobuf.at[g], wosem.at[g])

    def kv_start(n):
        b, g = where_is(n)
        s = slot(n)
        pltpu.make_async_copy(k_hbm.at[b, pl.ds(g * HG, HG)], kvbuf.at[s, 0], kvsem.at[s]).start()
        pltpu.make_async_copy(v_hbm.at[b, pl.ds(g * HG, HG)], kvbuf.at[s, 1], kvsem.at[s]).start()

    def kv_wait(n):
        s = slot(n)
        pltpu.make_async_copy(kvbuf.at[s], kvbuf.at[s], kvsem.at[s]).wait()

    def mm(a, w):
        return jnp.dot(a, w, preferred_element_type=jnp.float32)

    def qproj(n):
        b, g = where_is(n)
        return (mm(xbuf[b], wqbuf[g]) * scale).astype(jnp.bfloat16)

    def compute(n0, nh, toks, prefetch):
        b, g0 = where_is(n0)
        s0 = slot(n0)
        a = b % WARM_B
        nu = nh // HG
        qv, ps, ov, raw, st = {0: qs}, {}, {}, {}, {}

        def project(o, w, lo, hi, last, after):
            if after is not None:
                w0 = jnp.where(after < 0, 0.0, w[:16].astype(jnp.float32)).astype(w.dtype)
                w = jnp.concatenate([w0, w[16:]], axis=0)
            r = mm(o, w)
            new = st[lo] + r if lo in st else jnp.where(g0 == 0, r, acc[a, :, lo:hi] + r)
            st[lo] = new
            if last:
                acc[a, :, lo:hi] = new
                outbuf[b, :, lo:hi] = new.astype(outbuf.dtype)

        def group(u):
            return jnp.concatenate([ov[h] for h in range(u * HG, (u + 1) * HG)], axis=1)

        for ti, tok in enumerate(toks):
            after = None
            if tok.endswith("!"):
                tok = tok[:-1]
                after = jnp.max(jnp.abs(raw[nh - 1][Sq - 16:]), axis=1, keepdims=True)
            kind, n = tok[0], int(tok[1:])
            u, cols = n // HG, slice((n % HG) * DH, (n % HG + 1) * DH)
            if kind == "Q":
                s = lax.dot_general(qv[u][:, cols], kvbuf[s0 + u, 0, n % HG],
                                    (((1,), (1,)), ((), ())),
                                    preferred_element_type=jnp.float32)
                m = jnp.max(s, axis=1, keepdims=True)
                p = jnp.exp2(s - m).astype(jnp.bfloat16)
                l = jnp.sum(p.astype(jnp.float32), axis=1, keepdims=True)
                r = pl.reciprocal(l, approx=True)
                ps[n] = (p, r * (2.0 - l * r))
            elif kind == "P":
                p, r = ps.pop(n)
                raw[n] = mm(p, kvbuf[s0 + u, 1, n % HG])
                ov[n] = (raw[n] * r).astype(jnp.bfloat16)
            elif kind == "A":
                qv[n] = qproj(n0 + n)
            elif kind == "N":
                qs[...] = qproj(jnp.minimum(n0 + nu, NC - 1))
            elif kind == "c":
                project(ov[n], wobuf[g0 + u, cols, :W], 0, W, n == nh - 1, after)
            elif kind == "d":
                project(group(n), wobuf[g0 + n, :, W:], W, D, n == nu - 1, after)
            elif kind == "C":
                project(group(n), wobuf[g0 + n], 0, D, n == nu - 1, after)
            if ti == 1:
                prefetch()

        @pl.when(g0 == G - nu)
        def _():
            pltpu.make_async_copy(outbuf.at[b], o_hbm.at[b], osem).start()

    x_cp(0).start()
    wq_cp(0).start()
    kv_start(0)
    acc[...] = jnp.zeros(acc.shape, acc.dtype)
    x_cp(0).wait()
    wq_cp(0).wait()
    x_cp(1).start()
    wo_cp(0).start()
    kv_start(1)
    wq_cp(1).start()
    qs[...] = qproj(0)
    x_cp(1).wait()

    def warm_body(j, _):
        g = j // WARM_B
        first, last = j % WARM_B == 0, j % WARM_B == WARM_B - 1
        pl.when(first)(lambda: wo_cp(g).wait())
        pl.when(last & (g + 1 < G))(lambda: wq_cp(g + 1).wait())
        pl.when(j == J - 1)(lambda: x_cp(WARM_B).wait())
        kv_wait(j)

        def prefetch():
            na = j + 2 + sum((j > e).astype(jnp.int32) for e in LEAD_AT)
            extra = functools.reduce(jnp.logical_or, [j == e for e in LEAD_AT])
            pl.when(na < J + U)(lambda: kv_start(na))
            pl.when(extra)(lambda: kv_start(na + 1))
            pl.when(first & (g + 1 < G))(lambda: wo_cp(g + 1).start())
            pl.when(last & (g + 2 < G))(lambda: wq_cp(g + 2).start())
            pl.when(j == J - 3)(lambda: x_cp(WARM_B).start())

        compute(j, HG, WARM_ORDER, prefetch)

    lax.fori_loop(0, J, warm_body, None)

    def main_body(i, _):
        n0 = J + i * U
        b, g0 = where_is(n0)
        pl.when((g0 == G - U) & (b + 1 < B))(lambda: x_cp(b + 1).wait())
        for u in range(U):
            kv_wait(n0 + u)

        def prefetch():
            for u in range(U):
                pl.when(n0 + U + u < NC)(functools.partial(kv_start, n0 + U + u))
            pl.when((g0 == 0) & (b + 1 < B))(lambda: x_cp(b + 1).start())

        compute(n0, NH, _main_order(), prefetch)

    lax.fori_loop(0, (NC - J) // U, main_body, None)
    pltpu.make_async_copy(outbuf, o_hbm, osem).wait()


@jax.jit
def pallas_standalone__gqa_block_cached__near_ridge_kernel(
    x: jax.Array,
    k_cache: jax.Array,
    v_cache: jax.Array,
    wq: jax.Array,
    wo: jax.Array,
):
    B, Sq, D = x.shape
    _, H, Sk, _ = k_cache.shape
    assert k_cache.shape[3] == DH and wq.shape == (D, H * DH) and wo.shape == (H * DH, D)
    G = H // HG
    assert G == NSLOT == 2 * U and B > WARM_B
    bf = jnp.bfloat16
    hbm = pl.BlockSpec(memory_space=pl.ANY)
    return pl.pallas_call(
        _kernel,
        in_specs=[hbm] * 5,
        out_specs=hbm,
        out_shape=jax.ShapeDtypeStruct((B, Sq, D), x.dtype),
        scratch_shapes=[
            pltpu.VMEM((B, Sq, D), bf),
            pltpu.VMEM((G, D, W), bf),
            pltpu.VMEM((G, W, D), bf),
            pltpu.VMEM((NSLOT, 2, HG, Sk, DH), bf),
            pltpu.VMEM((Sq, W), bf),
            pltpu.VMEM((WARM_B, Sq, D), jnp.float32),
            pltpu.VMEM((B, Sq, D), x.dtype),
            pltpu.SemaphoreType.DMA((2,)),
            pltpu.SemaphoreType.DMA((G,)),
            pltpu.SemaphoreType.DMA((G,)),
            pltpu.SemaphoreType.DMA((NSLOT,)),
            pltpu.SemaphoreType.DMA,
        ],
        compiler_params=pltpu.CompilerParams(
            vmem_limit_bytes=100 * 1024 * 1024, disable_bounds_checks=True),
    )(x, k_cache, v_cache, wq, wo)
```

```python
import functools
import math

import jax
import jax.numpy as jnp
from jax import lax
import jax.experimental.pallas as pl
import jax.experimental.pallas.tpu as pltpu

DH = 128
HG = 4
W = HG * DH
NSLOT = 8
NH = 16
U = NH // HG
WARM_B = 2
LEAD_AT = (3, 7, 10, 13)

WARM_ORDER = "Q0 Q1 P0 Q2 P1 Q3 c0 P2 c1 P3 N0 c2 c3! d0".split()


def _main_order():
    toks = ["Q0"]
    for h in range(NH - 2):
        toks.append(f"Q{h + 1}")
        if (h + 2) % HG == 0:
            toks.append(f"A{(h + 2) // HG}")
        if h >= 2:
            toks.append(f"c{h - 2}")
            if (h - 2) % HG == HG - 1:
                toks.append(f"d{(h - 2) // HG}")
        toks.append(f"P{h}")
    n = NH
    return toks + [f"c{n - 4}", f"Q{n - 1}", f"P{n - 2}", f"c{n - 3}", f"P{n - 1}",
                   "N0", f"c{n - 2}", f"c{n - 1}!", f"d{U - 1}"]


def _kernel(x_hbm, k_hbm, v_hbm, wq_hbm, wo_hbm, o_hbm,
            xbuf, wqbuf, wobuf, kvbuf, qs, acc, outbuf,
            xsem, wqsem, wosem, kvsem, osem):
    B, Sq, D = x_hbm.shape
    G = k_hbm.shape[1] // HG
    NC = B * G
    J = WARM_B * G
    scale = (DH ** -0.5) * math.log2(math.e)

    def where_is(n):
        n = jnp.asarray(n, jnp.uint32)
        warm = n < J
        b = jnp.where(warm, n % WARM_B, n // G)
        g = jnp.where(warm, n // WARM_B, n % G)
        return b.astype(jnp.int32), g.astype(jnp.int32)

    def slot(n):
        return (jnp.asarray(n, jnp.uint32) % NSLOT).astype(jnp.int32)

    def x_cp(b):
        return pltpu.make_async_copy(x_hbm.at[b], xbuf.at[b], xsem.at[b % 2])

    def wq_cp(g):
        return pltpu.make_async_copy(
            wq_hbm.at[:, pl.ds(pl.multiple_of(g * W, W), W)], wqbuf.at[g], wqsem.at[g])

    def wo_cp(g):
        return pltpu.make_async_copy(
            wo_hbm.at[pl.ds(pl.multiple_of(g * W, W), W), :], wobuf.at[g], wosem.at[g])

    def kv_start(n):
        b, g = where_is(n)
        s = slot(n)
        pltpu.make_async_copy(k_hbm.at[b, pl.ds(g * HG, HG)], kvbuf.at[s, 0], kvsem.at[s]).start()
        pltpu.make_async_copy(v_hbm.at[b, pl.ds(g * HG, HG)], kvbuf.at[s, 1], kvsem.at[s]).start()

    def kv_wait(n):
        s = slot(n)
        pltpu.make_async_copy(kvbuf.at[s], kvbuf.at[s], kvsem.at[s]).wait()

    def mm(a, w):
        return jnp.dot(a, w, preferred_element_type=jnp.float32)

    def qproj(n):
        b, g = where_is(n)
        return (mm(xbuf[b], wqbuf[g]) * scale).astype(jnp.bfloat16)

    def compute(n0, nh, toks, prefetch):
        b, g0 = where_is(n0)
        s0 = slot(n0)
        a = b % WARM_B
        nu = nh // HG
        qv, ps, ov, raw, st = {0: qs}, {}, {}, {}, {}

        def project(o, w, lo, hi, last, after):
            if after is not None:
                w0 = jnp.where(after < 0, 0.0, w[:16].astype(jnp.float32)).astype(w.dtype)
                w = jnp.concatenate([w0, w[16:]], axis=0)
            r = mm(o, w)
            new = st[lo] + r if lo in st else jnp.where(g0 == 0, r, acc[a, :, lo:hi] + r)
            st[lo] = new
            if last:
                acc[a, :, lo:hi] = new
                outbuf[b, :, lo:hi] = new.astype(outbuf.dtype)

        def group(u):
            return jnp.concatenate([ov[h] for h in range(u * HG, (u + 1) * HG)], axis=1)

        for ti, tok in enumerate(toks):
            after = None
            if tok.endswith("!"):
                tok = tok[:-1]
                after = jnp.max(jnp.abs(raw[nh - 1][Sq - 16:]), axis=1, keepdims=True)
            kind, n = tok[0], int(tok[1:])
            u, cols = n // HG, slice((n % HG) * DH, (n % HG + 1) * DH)
            if kind == "Q":
                s = lax.dot_general(qv[u][:, cols], kvbuf[s0 + u, 0, n % HG],
                                    (((1,), (1,)), ((), ())),
                                    preferred_element_type=jnp.float32)
                m = jnp.max(s, axis=1, keepdims=True)
                p = jnp.exp2(s - m).astype(jnp.bfloat16)
                l = jnp.sum(p.astype(jnp.float32), axis=1, keepdims=True)
                r = pl.reciprocal(l, approx=True)
                ps[n] = (p, r * (2.0 - l * r))
            elif kind == "P":
                p, r = ps.pop(n)
                raw[n] = mm(p, kvbuf[s0 + u, 1, n % HG])
                ov[n] = (raw[n] * r).astype(jnp.bfloat16)
            elif kind == "A":
                qv[n] = qproj(n0 + n)
            elif kind == "N":
                qs[...] = qproj(jnp.minimum(n0 + nu, NC - 1))
            elif kind == "c":
                project(ov[n], wobuf[g0 + u, cols, :W], 0, W, n == nh - 1, after)
            elif kind == "d":
                project(group(n), wobuf[g0 + n, :, W:], W, D, n == nu - 1, after)
            if ti == 1:
                prefetch()

        @pl.when(g0 == G - nu)
        def _():
            pltpu.make_async_copy(outbuf.at[b], o_hbm.at[b], osem).start()

    x_cp(0).start()
    wq_cp(0).start()
    kv_start(0)
    acc[...] = jnp.zeros(acc.shape, acc.dtype)
    x_cp(0).wait()
    wq_cp(0).wait()
    x_cp(1).start()
    wo_cp(0).start()
    kv_start(1)
    wq_cp(1).start()
    qs[...] = qproj(0)
    x_cp(1).wait()

    def warm_body(j, _):
        g = j // WARM_B
        first, last = j % WARM_B == 0, j % WARM_B == WARM_B - 1
        pl.when(first)(lambda: wo_cp(g).wait())
        pl.when(last & (g + 1 < G))(lambda: wq_cp(g + 1).wait())
        pl.when(j == J - 1)(lambda: x_cp(WARM_B).wait())
        kv_wait(j)

        def prefetch():
            na = j + 2 + sum((j > e).astype(jnp.int32) for e in LEAD_AT)
            extra = functools.reduce(jnp.logical_or, [j == e for e in LEAD_AT])
            pl.when(na < J + U)(lambda: kv_start(na))
            pl.when(extra)(lambda: kv_start(na + 1))
            pl.when(first & (g + 1 < G))(lambda: wo_cp(g + 1).start())
            pl.when(last & (g + 2 < G))(lambda: wq_cp(g + 2).start())
            pl.when(j == J - 3)(lambda: x_cp(WARM_B).start())

        compute(j, HG, WARM_ORDER, prefetch)

    lax.fori_loop(0, J, warm_body, None)

    def main_body(i, _):
        n0 = J + i * U
        b, g0 = where_is(n0)
        pl.when((g0 == G - U) & (b + 1 < B))(lambda: x_cp(b + 1).wait())
        for u in range(U):
            kv_wait(n0 + u)

        def prefetch():
            for u in range(U):
                pl.when(n0 + U + u < NC)(functools.partial(kv_start, n0 + U + u))
            pl.when((g0 == 0) & (b + 1 < B))(lambda: x_cp(b + 1).start())

        compute(n0, NH, _main_order(), prefetch)

    lax.fori_loop(0, (NC - J) // U, main_body, None)
    pltpu.make_async_copy(outbuf, o_hbm, osem).wait()


@jax.jit
def pallas_standalone__gqa_block_cached__near_ridge_kernel(
    x: jax.Array,
    k_cache: jax.Array,
    v_cache: jax.Array,
    wq: jax.Array,
    wo: jax.Array,
):
    B, Sq, D = x.shape
    _, H, Sk, _ = k_cache.shape
    assert k_cache.shape[3] == DH and wq.shape == (D, H * DH) and wo.shape == (H * DH, D)
    G = H // HG
    assert G == NSLOT == 2 * U and B > WARM_B
    bf = jnp.bfloat16
    hbm = pl.BlockSpec(memory_space=pl.ANY)
    return pl.pallas_call(
        _kernel,
        in_specs=[hbm] * 5,
        out_specs=hbm,
        out_shape=jax.ShapeDtypeStruct((B, Sq, D), x.dtype),
        scratch_shapes=[
            pltpu.VMEM((B, Sq, D), bf),
            pltpu.VMEM((G, D, W), bf),
            pltpu.VMEM((G, W, D), bf),
            pltpu.VMEM((NSLOT, 2, HG, Sk, DH), bf),
            pltpu.VMEM((Sq, W), bf),
            pltpu.VMEM((WARM_B, Sq, D), jnp.float32),
            pltpu.VMEM((B, Sq, D), x.dtype),
            pltpu.SemaphoreType.DMA((2,)),
            pltpu.SemaphoreType.DMA((G,)),
            pltpu.SemaphoreType.DMA((G,)),
            pltpu.SemaphoreType.DMA((NSLOT,)),
            pltpu.SemaphoreType.DMA,
        ],
        compiler_params=pltpu.CompilerParams(
            vmem_limit_bytes=100 * 1024 * 1024, disable_bounds_checks=True),
    )(x, k_cache, v_cache, wq, wo)
```
